```python
import os as _os
_os.environ.setdefault("JAX_PLATFORMS", "cpu")
import jax
import jax.numpy as jnp

def _softmax(x, axis=-1):
    return jax.nn.softmax(x, axis=axis)
def _gelu(x):
    return jax.nn.gelu(x, approximate=True)
def _silu(x):
    return jax.nn.silu(x)
def _sigmoid(x):
    return jax.nn.sigmoid(x)
def _layernorm(x, axis=-1, eps=1e-5):
    m = jnp.mean(x, axis=axis, keepdims=True)
    v = jnp.var(x, axis=axis, keepdims=True)
    return (x - m) / jnp.sqrt(v + eps)
def _scatter_add(tgt, idx, src, axis=0):
    return tgt.at[idx].add(src)
def _segment_sum(src, seg, n):
    return jax.ops.segment_sum(src, seg, n)
class _Rng:
    def __init__(self, key):
        self._k = key
    def _next(self):
        self._k, sub = jax.random.split(self._k)
        return sub
    def normal(self, shape):
        return jax.random.normal(self._next(), shape, dtype=jnp.bfloat16)
    def randint(self, lo, hi, shape):
        return jax.random.randint(self._next(), shape, lo, hi, dtype=jnp.int32)
    def uniform(self, shape, lo=0.0, hi=1.0):
        return jax.random.uniform(self._next(), shape, jnp.bfloat16, lo, hi)
    def permutation(self, n):
        return jax.random.permutation(self._next(), n)


kernel_name = 'concat_heads__gqa_block_cached__gqa_block_cached__near_ridge'

def setup_inputs():
    _rng = _Rng(jax.random.key(int.from_bytes(__import__("os").urandom(4), "little")))
    _w = (lambda a: (lambda t: t.astype(jnp.bfloat16) if jnp.issubdtype(t.dtype, jnp.floating) else t)(jnp.asarray(a)))
    def _A_setup():
        B, Sq, D = 16, 144, 448
        Hq, Hkv, Sk, Dh = 16, 8, 1024, 256
        assert Hq % Hkv == 0, (Hq, Hkv)
        return {
            "x": _w((lambda *s: _rng.normal(s) * 0.8)(B, Sq, D)),
            "k_cache": _w((lambda *s: _rng.normal(s) * 0.8)(B, Hkv, Sk, Dh)),
            "v_cache": _w((lambda *s: _rng.normal(s) * 0.05)(B, Hkv, Sk, Dh)),
            "wq": _w((lambda *s: _rng.normal(s) * 0.8)(D, Hq * Dh) * (D ** -0.5)),
            "wo": _w((lambda *s: _rng.normal(s) * 0.05)(Hq * Dh, D) * ((Hq * Dh) ** -0.5)),
        }
    _A_in = _A_setup()

    def _B_setup():
        B, Sq, D = 16, 144, 448
        Hq, Hkv, Sk, Dh = 16, 8, 1024, 256
        assert Hq % Hkv == 0, (Hq, Hkv)
        return {
            "x": _w((lambda *s: _rng.normal(s) * 0.8)(B, Sq, D)),
            "k_cache": _w((lambda *s: _rng.normal(s) * 0.8)(B, Hkv, Sk, Dh)),
            "v_cache": _w((lambda *s: _rng.normal(s) * 0.05)(B, Hkv, Sk, Dh)),
            "wq": _w((lambda *s: _rng.normal(s) * 0.8)(D, Hq * Dh) * (D ** -0.5)),
            "wo": _w((lambda *s: _rng.normal(s) * 0.05)(Hq * Dh, D) * ((Hq * Dh) ** -0.5)),
        }
    _B_in = _B_setup()

    return {
        "A_x": _A_in["x"],
        "A_k_cache": _A_in["k_cache"],
        "A_v_cache": _A_in["v_cache"],
        "A_wq": _A_in["wq"],
        "A_wo": _A_in["wo"],
        "B_x": _B_in["x"],
        "B_k_cache": _B_in["k_cache"],
        "B_v_cache": _B_in["v_cache"],
        "B_wq": _B_in["wq"],
        "B_wo": _B_in["wo"],
    }

def reference(A_x, A_k_cache, A_v_cache, A_wq, A_wo, B_x, B_k_cache, B_v_cache, B_wq, B_wo):
    def _A_ref(x, k_cache, v_cache, wq, wo):
        B, Sq, D = x.shape
        Hq, Dh = 16, 256
        Hkv = k_cache.shape[1]
        rep = Hq // Hkv
        q = (lambda x, *d: x.transpose(*d))((x @ wq).reshape(B, Sq, Hq, Dh), 0, 2, 1, 3)
        k = jnp.repeat(k_cache, rep, axis=1)
        v = jnp.repeat(v_cache, rep, axis=1)
        scores = jnp.einsum("bhqd,bhkd->bhqk", q, k) * (Dh ** -0.5)
        p = _softmax(scores, axis=-1)
        o = jnp.einsum("bhqk,bhkd->bhqd", p, v)
        return (lambda x, *d: x.transpose(*d))(o, 0, 2, 1, 3).reshape(B, Sq, Hq * Dh) @ wo

    def _B_ref(x, k_cache, v_cache, wq, wo):
        B, Sq, D = x.shape
        Hq, Dh = 16, 256
        Hkv = k_cache.shape[1]
        rep = Hq // Hkv
        q = (lambda x, *d: x.transpose(*d))((x @ wq).reshape(B, Sq, Hq, Dh), 0, 2, 1, 3)
        k = jnp.repeat(k_cache, rep, axis=1)
        v = jnp.repeat(v_cache, rep, axis=1)
        scores = jnp.einsum("bhqd,bhkd->bhqk", q, k) * (Dh ** -0.5)
        p = _softmax(scores, axis=-1)
        o = jnp.einsum("bhqk,bhkd->bhqd", p, v)
        return (lambda x, *d: x.transpose(*d))(o, 0, 2, 1, 3).reshape(B, Sq, Hq * Dh) @ wo

    a = _A_ref(A_x, A_k_cache, A_v_cache, A_wq, A_wo)
    b = _B_ref(B_x, B_k_cache, B_v_cache, B_wq, B_wo)
    return jnp.concatenate([a, b], axis=-1)
```

```python
import functools
import jax
import jax.numpy as jnp
from jax import lax
import jax.experimental.pallas as pl
import jax.experimental.pallas.tpu as pltpu

B, SQ, D, HQ, HKV, SK, DH = 16, 144, 448, 16, 8, 1024, 256
REP = HQ // HKV
GW = REP * DH
T = B * SQ
TT = 128
NT = (((1,), (1,)), ((), ()))
C = 1.4426950408889634 * DH ** -0.5


def _attend(q, k, v, sm=0, KC=256):
    s = lax.dot_general(q, k, NT, preferred_element_type=jnp.float32)
    m = jnp.max(s, axis=-1, keepdims=True)
    o = l = None
    for c in range(0, SK, KC):
        p = jnp.exp2(s[:, c:c + KC] - m)
        pb = p.astype(jnp.bfloat16)
        ps = pb.astype(jnp.float32) if sm else p
        for t in range(0, KC, 128):
            l = ps[:, t:t + 128] if l is None else l + ps[:, t:t + 128]
        t = jnp.dot(pb, v[c:c + KC], preferred_element_type=jnp.float32)
        o = t if o is None else o + t
    return o, l


def kernel(xa, ka, va, wqa, woa, xb, kb, vb, wqb, wob, out,
           x_buf, wq_buf, wo_buf, k_buf, v_buf, q_buf, o_buf, acc_buf, l_buf, out_buf,
           x_sem, wq_sem, wo_sem, k_sem, v_sem, out_sem, *, U, NS, PU, PH, QU, QR, nodma=False, **akw):
    x_hbm, k_hbm, v_hbm, wq_hbm, wo_hbm = (xa, xb), (ka, kb), (va, vb), (wqa, wqb), (woa, wob)
    NB = B // U
    NIT = HKV * NB
    NQ = B // QU

    def x_copy(br, j):
        rows = pl.ds(pl.multiple_of(j * (QU * SQ), 16), QU * SQ)
        return pltpu.make_async_copy(x_hbm[br].at[rows], x_buf.at[br, rows], x_sem.at[br, j])

    def wq_copy(br, g):
        return pltpu.make_async_copy(
            wq_hbm[br].at[:, pl.ds(pl.multiple_of(g * GW, GW), GW)], wq_buf.at[br, g], wq_sem.at[br, g])

    def wo_copy(br):
        return pltpu.make_async_copy(wo_hbm[br], wo_buf.at[br], wo_sem.at[br])

    def k_copy(br, it, slot):
        return pltpu.make_async_copy(
            k_hbm[br].at[pl.ds((it % NB) * U, U), it // NB], k_buf.at[slot, br], k_sem.at[slot, br])

    def v_copy(br, it, slot):
        return pltpu.make_async_copy(
            v_hbm[br].at[pl.ds((it % NB) * U, U), it // NB], v_buf.at[slot, br], v_sem.at[slot, br])

    def kv_copies(it, slot):
        return [f(br, it, slot) for br in range(2) for f in (k_copy, v_copy)]

    def project_q(g, b0, n, brs=(0, 1)):
        r0 = pl.multiple_of(b0 * SQ, 16)
        for br in brs:
            q = jnp.dot(x_buf[br, pl.ds(r0, n * SQ)], wq_buf[br, g], preferred_element_type=jnp.float32)
            q = (q * C).astype(jnp.bfloat16)
            for u in range(n):
                for h in range(REP):
                    q_buf[g % QR, br, b0 + u, h * SQ:(h + 1) * SQ] = q[u * SQ:(u + 1) * SQ, h * DH:(h + 1) * DH]

    def normalize(it):
        g, b0 = it // NB, (it % NB) * U
        r0 = pl.multiple_of(b0 * SQ, 16)
        for n in range(2 * U):
            br, u = divmod(n, U)
            l = jnp.sum(l_buf[n], axis=-1, keepdims=True)
            r = pl.reciprocal(l, approx=True)
            r = r * (2.0 - l * r)
            o = (acc_buf[n] * r).astype(jnp.bfloat16)
            for h in range(REP):
                o_buf[br, g, pl.ds(r0 + u * SQ, SQ), h * DH:(h + 1) * DH] = o[h * SQ:(h + 1) * SQ]

    def attend(it, slot, project):
        g, b0 = it // NB, (it % NB) * U
        normalize((it + NIT - 1) % NIT)
        for n in range(2 * U):
            br, u = divmod(n, U)
            acc_buf[n], l_buf[n] = _attend(q_buf[g % QR, br, b0 + u], k_buf[slot, br, u], v_buf[slot, br, u], **akw)
        if project:
            project_q(g + PH, b0, U)

    for br in range(2):
        x_copy(br, 0).start()
        wq_copy(br, 0).start()
    acc_buf[...] = jnp.zeros_like(acc_buf)
    l_buf[...] = jnp.ones_like(l_buf)
    for br in range(2):
        x_copy(br, 0).wait()
        wq_copy(br, 0).wait()
    for br in range(2):
        x_copy(br, 1).start()
        wq_copy(br, 1).start()

    def pre_step(i, carry):
        project_q(i // NQ, (i % NQ) * QU, QU)

        @pl.when(i + 1 < NQ)
        def _():
            for br in range(2):
                x_copy(br, i + 1).wait()

        @pl.when(i + 2 < NQ)
        def _():
            for br in range(2):
                x_copy(br, i + 2).start()

        @pl.when(i + 2 == NQ)
        def _():
            for c in kv_copies(0, 0):
                c.start()
            for g in range(2, PH + 1):
                for br in range(2):
                    wq_copy(br, g).start()

        @pl.when(i % NQ == NQ - 1)
        def _():
            for br in range(2):
                wq_copy(br, i // NQ + 1).wait()
        return carry

    lax.fori_loop(0, PH * NQ, pre_step, 0)
    for c in kv_copies(0, 0):
        c.wait()
    if not nodma:
        for s in range(1, NS):
            for c in kv_copies(s, s):
                c.start()

    def attn_step(it, slot, project):
        g, j = it // NB, it % NB
        attend(it, 0 if nodma else slot, project)

        nslot = jnp.where(slot == NS - 1, 0, slot + 1)
        if not nodma:
            @pl.when(it + NS < NIT)
            def _():
                for c in kv_copies(it + NS, slot):
                    c.start()

        if project:
            @pl.when(jnp.logical_and(j == 0, g + PH + 1 < HKV))
            def _():
                for br in range(2):
                    wq_copy(br, g + PH + 1).start()

            for br in range(2):
                @pl.when(it == (br + 1) * NB)
                def _():
                    wo_copy(br).start()

            @pl.when(jnp.logical_and(j == NB - 1, g + PH + 1 < HKV))
            def _():
                for br in range(2):
                    wq_copy(br, g + PH + 1).wait()

        if not nodma:
            @pl.when(it + 1 < NIT)
            def _():
                for c in kv_copies(it + 1, nslot):
                    c.wait()
        return nslot

    N1 = (HKV - PH) * NB
    lax.fori_loop(0, N1, functools.partial(attn_step, project=True), 0)
    lax.fori_loop(N1, NIT, functools.partial(attn_step, project=False), N1 % NS)

    normalize(NIT - 1)

    for br in range(2):
        wo_copy(br).wait()

    def out_copy(t, slot):
        rows = pl.ds(pl.multiple_of(t * (PU * TT), TT), PU * TT)
        return pltpu.make_async_copy(out_buf.at[slot], out.at[rows], out_sem.at[slot])

    NPS = T // (PU * TT)

    def proj_step(t, carry):
        slot = t % 2
        for i in range(PU):
            r0 = pl.multiple_of((t * PU + i) * TT, TT)
            parts = []
            for br in range(2):
                o = jnp.concatenate([o_buf[br, g, pl.ds(r0, TT)] for g in range(HKV)], axis=1)
                parts.append(lax.dot_general(wo_buf[br], o, NT, preferred_element_type=jnp.float32))
            out_buf[slot, i * TT:(i + 1) * TT] = jnp.concatenate(parts, axis=0).T.astype(out_buf.dtype)
        out_copy(t, slot).start()

        @pl.when(t >= 1)
        def _():
            out_copy(t - 1, 1 - slot).wait()
        return carry

    lax.fori_loop(0, NPS, proj_step, 0)
    out_copy(NPS - 1, (NPS - 1) % 2).wait()


def impl(A_x, A_k, A_v, A_wq, A_wo, B_x, B_k, B_v, B_wq, B_wo, U=4, NS=3, PU=3, PH=2, QU=4, QR=2, flags=None, nobc=True, **kw):
    bf = jnp.bfloat16
    hbm = pl.BlockSpec(memory_space=pltpu.HBM)
    res = pl.pallas_call(
        functools.partial(kernel, U=U, NS=NS, PU=PU, PH=PH, QU=QU, QR=QR, **kw),
        in_specs=[hbm] * 10,
        out_specs=hbm,
        out_shape=jax.ShapeDtypeStruct((T, 2 * D), bf),
        scratch_shapes=[
            pltpu.VMEM((2, T, D), bf),
            pltpu.VMEM((2, HKV, D, GW), bf),
            pltpu.VMEM((2, D, HQ * DH), bf),
            pltpu.VMEM((NS, 2, U, SK, DH), bf),
            pltpu.VMEM((NS, 2, U, SK, DH), bf),
            pltpu.VMEM((QR, 2, B, REP * SQ, DH), bf),
            pltpu.VMEM((2, HKV, T, GW), bf),
            pltpu.VMEM((2 * U, REP * SQ, DH), jnp.float32),
            pltpu.VMEM((2 * U, REP * SQ, 128), jnp.float32),
            pltpu.VMEM((2, PU * TT, 2 * D), bf),
            pltpu.SemaphoreType.DMA((2, B // QU)),
            pltpu.SemaphoreType.DMA((2, HKV)),
            pltpu.SemaphoreType.DMA((2,)),
            pltpu.SemaphoreType.DMA((NS, 2)),
            pltpu.SemaphoreType.DMA((NS, 2)),
            pltpu.SemaphoreType.DMA((2,)),
        ],
        compiler_params=pltpu.CompilerParams(
            vmem_limit_bytes=124 * 2**20, flags=flags, disable_bounds_checks=nobc),
    )(A_x.reshape(T, D), A_k, A_v, A_wq, A_wo.T, B_x.reshape(T, D), B_k, B_v, B_wq, B_wo.T)
    return res.reshape(B, SQ, 2 * D)


@jax.jit
def pallas_concat_heads__gqa_block_cached__gqa_block_cached__near_ridge_kernel(
        A_x, A_k_cache, A_v_cache, A_wq, A_wo, B_x, B_k_cache, B_v_cache, B_wq, B_wo):
    return impl(A_x, A_k_cache, A_v_cache, A_wq, A_wo, B_x, B_k_cache, B_v_cache, B_wq, B_wo)
```

```python
import functools

import jax
import jax.numpy as jnp
from jax import lax
import jax.experimental.pallas as pl
import jax.experimental.pallas.tpu as pltpu

B, SQ, D, HQ, HKV, SK, DH = 16, 144, 448, 16, 8, 1024, 256
REP = HQ // HKV
GW = REP * DH
T = B * SQ

U = 4
NB = B // U
NIT = HKV * NB
PH = 2
NS = 3
KC = 256
TT = 128
NTILE = T // TT
PU = 2

Q_SCALE = 1.4426950408889634 * DH ** -0.5
NT = (((1,), (1,)), ((), ()))


def _attend(q, k, v):
    s = lax.dot_general(q, k, NT, preferred_element_type=jnp.float32)
    m = jnp.max(s, axis=-1, keepdims=True)
    o = l = None
    for c in range(0, SK, KC):
        p = jnp.exp2(s[:, c:c + KC] - m)
        for t in range(0, KC, 128):
            l = p[:, t:t + 128] if l is None else l + p[:, t:t + 128]
        pv = jnp.dot(p.astype(v.dtype), v[c:c + KC], preferred_element_type=jnp.float32)
        o = pv if o is None else o + pv
    return o, l


def _kernel(xa, ka, va, wqa, woa, xb, kb, vb, wqb, wob, out,
            x_buf, wq_buf, wo_buf, k_buf, v_buf, q_buf, o_buf, acc_buf, l_buf, t_buf, out_buf,
            x_sem, wq_sem, wo_sem, k_sem, v_sem, out_sem):
    x_hbm, k_hbm, v_hbm = (xa, xb), (ka, kb), (va, vb)
    wq_hbm, wo_hbm = (wqa, wqb), (woa, wob)
    both = (0, 1)

    def x_copy(br, j):
        rows = pl.ds(j * U * SQ, U * SQ)
        return pltpu.make_async_copy(x_hbm[br].at[rows], x_buf.at[br, rows], x_sem.at[br, j])

    def wq_copy(br, g):
        cols = pl.ds(pl.multiple_of(g * GW, GW), GW)
        return pltpu.make_async_copy(wq_hbm[br].at[:, cols], wq_buf.at[br, g], wq_sem.at[br, g])

    def wo_copy(br):
        return pltpu.make_async_copy(wo_hbm[br], wo_buf.at[br], wo_sem.at[br])

    def kv_copies(it, slot):
        batches, g = pl.ds((it % NB) * U, U), it // NB
        return [
            pltpu.make_async_copy(hbm[br].at[batches, g], buf.at[slot, br], sem.at[slot, br])
            for br in both
            for hbm, buf, sem in ((k_hbm, k_buf, k_sem), (v_hbm, v_buf, v_sem))
        ]

    def out_copy(tile):
        rows = pl.ds(pl.multiple_of(tile * TT, TT), TT)
        return pltpu.make_async_copy(out_buf.at[rows], out.at[rows], out_sem.at[tile])

    def project_q(g, b0, branches=both):
        rows = pl.ds(pl.multiple_of(b0 * SQ, 16), U * SQ)
        for br in branches:
            q = jnp.dot(x_buf[br, rows], wq_buf[br, g], preferred_element_type=jnp.float32)
            q = (q * Q_SCALE).astype(q_buf.dtype)
            for u in range(U):
                for h in range(REP):
                    q_buf[g % PH, br, b0 + u, h * SQ:(h + 1) * SQ] = (
                        q[u * SQ:(u + 1) * SQ, h * DH:(h + 1) * DH])

    def normalize(it, br, u):
        g, b = it // NB, (it % NB) * U + u
        l = jnp.sum(l_buf[br, u], axis=-1, keepdims=True)
        r = pltpu.reciprocal(l, approx=True)
        r = r * (2.0 - l * r)
        o = (acc_buf[br, u] * r).astype(o_buf.dtype)
        rows = pl.ds(pl.multiple_of(b * SQ, 16), SQ)
        for h in range(REP):
            o_buf[br, g, rows, h * DH:(h + 1) * DH] = o[h * SQ:(h + 1) * SQ]

    assert PH == 2 and NB == 4
    wq_copy(0, 0).start()
    x_copy(0, 0).start()
    acc_buf[...] = jnp.zeros_like(acc_buf)
    l_buf[...] = jnp.ones_like(l_buf)
    t_buf[...] = jnp.zeros_like(t_buf)
    wq_copy(0, 0).wait()
    wq_copy(1, 0).start()
    x_copy(1, 0).start()
    wq_copy(0, 1).start()
    x_copy(0, 0).wait()
    project_q(0, 0, (0,))
    wq_copy(1, 0).wait()
    wq_copy(1, 1).start()
    x_copy(1, 0).wait()
    project_q(0, 0, (1,))
    for br in both:
        wq_copy(br, 1).wait()
    for br in both:
        x_copy(br, 1).start()

    def query_step(i, carry):
        project_q(i % PH, (i // PH) * U)

        @pl.when(i == 2)
        def _():
            for c in kv_copies(0, 0):
                c.start()

        @pl.when(i == 1)
        def _():
            for br in both:
                x_copy(br, 1).wait()
            for j in (2, 3):
                for br in both:
                    x_copy(br, j).start()

        @pl.when(i == 3)
        def _():
            for j in (2, 3):
                for br in both:
                    x_copy(br, j).wait()
            for br in both:
                wq_copy(br, PH).start()

        return carry

    lax.fori_loop(1, PH * NB, query_step, 0)
    for br in both:
        wq_copy(br, PH).wait()
    for c in kv_copies(0, 0):
        c.wait()
    for s in range(1, NS):
        for c in kv_copies(s, s):
            c.start()

    def attention_step(it, slot, project):
        g, j = it // NB, it % NB
        for br in both:
            for u in range(U):
                normalize((it + NIT - 1) % NIT, br, u)
        for br in both:
            for u in range(U):
                acc_buf[br, u], l_buf[br, u] = _attend(
                    q_buf[g % PH, br, j * U + u], k_buf[slot, br, u], v_buf[slot, br, u])
        if project:
            project_q(g + PH, j * U)

        @pl.when(it + NS < NIT)
        def _():
            for c in kv_copies(it + NS, slot):
                c.start()

        if project:
            @pl.when(jnp.logical_and(j == 0, g + PH + 1 < HKV))
            def _():
                for br in both:
                    wq_copy(br, g + PH + 1).start()

            for br in both:
                pl.when(it == (br + 1) * NB)(wo_copy(br).start)

            @pl.when(jnp.logical_and(j == NB - 1, g + PH + 1 < HKV))
            def _():
                for br in both:
                    wq_copy(br, g + PH + 1).wait()

        next_slot = jnp.where(slot == NS - 1, 0, slot + 1)

        @pl.when(it + 1 < NIT)
        def _():
            for c in kv_copies(it + 1, next_slot):
                c.wait()

        return next_slot

    n1 = (HKV - PH) * NB
    lax.fori_loop(0, n1, functools.partial(attention_step, project=True), 0)
    lax.fori_loop(n1, NIT, functools.partial(attention_step, project=False), n1 % NS)

    for br in both:
        wo_copy(br).wait()

    def emit(tile, out_t):
        out_buf[pl.ds(pl.multiple_of(tile * TT, TT), TT)] = out_t.T.astype(out_buf.dtype)

    def output_step(t, carry):
        late = (t * PU + NTILE - 1) % NTILE
        emit(late, t_buf[...])
        pl.when(t > 0)(out_copy(late).start)
        for i in range(PU):
            tile = t * PU + i
            rows = pl.ds(pl.multiple_of(tile * TT, TT), TT)
            out_t = jnp.concatenate([
                lax.dot_general(
                    wo_buf[br],
                    jnp.concatenate([o_buf[br, g, rows] for g in range(HKV)], axis=1),
                    NT, preferred_element_type=jnp.float32)
                for br in both], axis=0)
            if i < PU - 1:
                emit(tile, out_t)
                out_copy(tile).start()
            else:
                t_buf[...] = out_t
        n = jnp.minimum(t, 2 * U - 1)
        normalize(NIT - 1, n % 2, n // 2)

        for i in range(PU):
            done = (t - 1) * PU - 1 + i
            pl.when(done >= 0)(lambda: out_copy(done).wait())
        return carry

    assert U == 4 and PU == 2
    lax.fori_loop(0, NTILE // PU, output_step, 0)
    emit(NTILE - 1, t_buf[...])
    out_copy(NTILE - 1).start()
    for tile in range(NTILE - PU - 1, NTILE):
        out_copy(tile).wait()


@jax.jit
def pallas_concat_heads__gqa_block_cached__gqa_block_cached__near_ridge_kernel(
    A_x: jax.Array,
    A_k_cache: jax.Array,
    A_v_cache: jax.Array,
    A_wq: jax.Array,
    A_wo: jax.Array,
    B_x: jax.Array,
    B_k_cache: jax.Array,
    B_v_cache: jax.Array,
    B_wq: jax.Array,
    B_wo: jax.Array,
):
    dt = A_x.dtype
    hbm = pl.BlockSpec(memory_space=pltpu.HBM)
    out = pl.pallas_call(
        _kernel,
        in_specs=[hbm] * 10,
        out_specs=hbm,
        out_shape=jax.ShapeDtypeStruct((T, 2 * D), dt),
        scratch_shapes=[
            pltpu.VMEM((2, T, D), dt),
            pltpu.VMEM((2, HKV, D, GW), dt),
            pltpu.VMEM((2, D, HQ * DH), dt),
            pltpu.VMEM((NS, 2, U, SK, DH), dt),
            pltpu.VMEM((NS, 2, U, SK, DH), dt),
            pltpu.VMEM((PH, 2, B, REP * SQ, DH), dt),
            pltpu.VMEM((2, HKV, T, GW), dt),
            pltpu.VMEM((2, U, REP * SQ, DH), jnp.float32),
            pltpu.VMEM((2, U, REP * SQ, 128), jnp.float32),
            pltpu.VMEM((2 * D, TT), jnp.float32),
            pltpu.VMEM((T, 2 * D), dt),
            pltpu.SemaphoreType.DMA((2, NB)),
            pltpu.SemaphoreType.DMA((2, HKV)),
            pltpu.SemaphoreType.DMA((2,)),
            pltpu.SemaphoreType.DMA((NS, 2)),
            pltpu.SemaphoreType.DMA((NS, 2)),
            pltpu.SemaphoreType.DMA((NTILE,)),
        ],
        compiler_params=pltpu.CompilerParams(
            vmem_limit_bytes=124 * 2**20, disable_bounds_checks=True),
    )(
        A_x.reshape(T, D), A_k_cache, A_v_cache, A_wq, A_wo.T,
        B_x.reshape(T, D), B_k_cache, B_v_cache, B_wq, B_wo.T,
    )
    return out.reshape(B, SQ, 2 * D)
```
